```python
import os as _os
_os.environ.setdefault("JAX_PLATFORMS", "cpu")
import jax
import jax.numpy as jnp

def _softmax(x, axis=-1):
    return jax.nn.softmax(x, axis=axis)
def _gelu(x):
    return jax.nn.gelu(x, approximate=True)
def _silu(x):
    return jax.nn.silu(x)
def _sigmoid(x):
    return jax.nn.sigmoid(x)
def _layernorm(x, axis=-1, eps=1e-5):
    m = jnp.mean(x, axis=axis, keepdims=True)
    v = jnp.var(x, axis=axis, keepdims=True)
    return (x - m) / jnp.sqrt(v + eps)
def _scatter_add(tgt, idx, src, axis=0):
    return tgt.at[idx].add(src)
def _segment_sum(src, seg, n):
    return jax.ops.segment_sum(src, seg, n)
class _Rng:
    def __init__(self, key):
        self._k = key
    def _next(self):
        self._k, sub = jax.random.split(self._k)
        return sub
    def normal(self, shape):
        return jax.random.normal(self._next(), shape, dtype=jnp.bfloat16)
    def randint(self, lo, hi, shape):
        return jax.random.randint(self._next(), shape, lo, hi, dtype=jnp.int32)
    def uniform(self, shape, lo=0.0, hi=1.0):
        return jax.random.uniform(self._next(), shape, jnp.bfloat16, lo, hi)
    def permutation(self, n):
        return jax.random.permutation(self._next(), n)


kernel_name = 'standalone__sliding_local_fixed_window__prompt'

def setup_inputs():
    _rng = _Rng(jax.random.key(int.from_bytes(__import__("os").urandom(4), "little")))
    _w = (lambda a: (lambda t: t.astype(jnp.bfloat16) if jnp.issubdtype(t.dtype, jnp.floating) else t)(jnp.asarray(a)))
    B, H, S, D = 1, 32, 2048, 128
    return {
        "q": _w((lambda *s: _rng.normal(s) * 0.4)(B, H, S, D)),
        "k": _w((lambda *s: _rng.normal(s) * 0.4)(B, H, S, D)),
        "v": _w((lambda *s: _rng.normal(s) * 0.05)(B, H, S, D)),
    }

def reference(q, k, v):
    B, H, S, D = q.shape
    w = 32
    pos = jnp.arange(S)
    rel = pos[:, None] - pos[None, :]
    mask = (rel >= 0) & (rel < w)
    scores = jnp.einsum("bhqd,bhkd->bhqk", q, k) * (D ** -0.5)
    scores = jnp.where(mask[None, None], scores, (lambda x, dt: x.astype(dt))(jnp.array(-1e9), q.dtype))
    p = _softmax(scores, axis=-1)
    return jnp.einsum("bhqk,bhkd->bhqd", p, v)
```

```python
import functools
import math

import jax
import jax.numpy as jnp
from jax import lax
import jax.experimental.pallas as pl
import jax.experimental.pallas.tpu as pltpu

WINDOW = 32
KT = 128
TQ = KT - WINDOW
NEG = -1e30
WRITE_ROWS = 64
TAIL_ROWS = 1536


def _chunk_sizes(num_heads):
    n = max(1, num_heads // 4)
    sizes = [n] * (num_heads // n)
    if num_heads % n:
        sizes.append(num_heads % n)
    return sizes


@jax.jit
def pallas_standalone__sliding_local_fixed_window__prompt_kernel(
    q: jax.Array,
    k: jax.Array,
    v: jax.Array,
):
    B, H, S, D = q.shape
    NH = B * H
    assert D == 128 and S >= KT and (S - KT) % TQ == 0 and S % WRITE_ROWS == 0
    assert S > TAIL_ROWS and NH >= 4
    q3, k3, v3 = (x.reshape(NH, S, D) for x in (q, k, v))

    chunks = _chunk_sizes(NH)
    nch = len(chunks)
    starts = [sum(chunks[:c]) for c in range(nch)]
    last0 = starts[-1]
    nblk = (S - KT) // TQ
    c1 = (D ** -0.5) * math.log2(math.e)

    def kernel(q_hbm, k_hbm, v_hbm, o_hbm, qb, kb, vb, ob, bias0_ref, bias_ref,
               rsems, wsem):
        def read_copies(c):
            h0, n = starts[c], chunks[c]
            sem = rsems.at[c]
            hs = pl.ds(h0, n)
            cps = [pltpu.make_async_copy(q_hbm.at[hs], qb.at[hs], sem),
                   pltpu.make_async_copy(k_hbm.at[hs], kb.at[hs], sem)]
            if c < nch - 1:
                cps.append(pltpu.make_async_copy(v_hbm.at[hs], vb.at[hs], sem))
            else:
                if n > 1:
                    hs1 = pl.ds(h0, n - 1)
                    cps.append(
                        pltpu.make_async_copy(v_hbm.at[hs1], vb.at[hs1], sem))
                rs = pl.ds(0, S - TAIL_ROWS)
                cps.append(pltpu.make_async_copy(
                    v_hbm.at[NH - 1, rs], vb.at[NH - 1, rs], sem))
            return cps

        def tail_copy():
            rs = pl.ds(S - TAIL_ROWS, TAIL_ROWS)
            return pltpu.make_async_copy(
                v_hbm.at[NH - 1, rs], vb.at[NH - 1, rs], rsems.at[nch])

        def write_copies(h0, n):
            hs = pl.ds(h0, n)
            return [
                pltpu.make_async_copy(
                    ob.at[hs, pl.ds(j * WRITE_ROWS, WRITE_ROWS)],
                    o_hbm.at[hs, pl.ds(j * WRITE_ROWS, WRITE_ROWS)], wsem)
                for j in range(S // WRITE_ROWS)
            ]

        for c in range(nch):
            for cp in read_copies(c):
                cp.start()
        tail_copy().start()

        row = lax.broadcasted_iota(jnp.int32, (KT, KT), 0)
        col = lax.broadcasted_iota(jnp.int32, (KT, KT), 1)
        rel0 = row - col
        bias0_ref[...] = jnp.where((rel0 >= 0) & (rel0 < WINDOW), 0.0, NEG)
        rel = rel0 + WINDOW
        bias_ref[...] = jnp.where((rel >= 0) & (rel < WINDOW), 0.0, NEG)

        def block(h, q0, nq, k0, bias):
            qq = qb[h, pl.ds(q0, nq), :]
            kk = kb[h, pl.ds(k0, KT), :]
            vv = vb[h, pl.ds(k0, KT), :]
            s = lax.dot_general(qq, kk, (((1,), (1,)), ((), ())),
                                preferred_element_type=jnp.float32)
            s = s + bias
            m = jnp.max(s, axis=-1, keepdims=True)
            p = jnp.exp2((s - m) * c1)
            l = jnp.sum(p, axis=-1, keepdims=True)
            o = jnp.dot(p.astype(vv.dtype), vv,
                        preferred_element_type=jnp.float32)
            ob[h, pl.ds(q0, nq), :] = (o / l).astype(ob.dtype)

        def arrive(c):
            for cp in read_copies(c):
                cp.wait()
            if c == nch - 1:
                for cp in write_copies(0, last0):
                    cp.start()

        def head(h, carry):
            for c in range(nch):
                pl.when(h == starts[c])(functools.partial(arrive, c))

            @pl.when(h == NH - 1)
            def _():
                tail_copy().wait()

            block(h, 0, KT, 0, bias0_ref[...])
            for j in range(nblk):
                q0 = KT + j * TQ
                block(h, q0, TQ, q0 - WINDOW, bias_ref[0:TQ, :])
            return carry

        lax.fori_loop(0, NH, head, 0)

        for cp in write_copies(last0, NH - last0):
            cp.start()
        for cp in write_copies(0, last0) + write_copies(last0, NH - last0):
            cp.wait()

    any_spec = pl.BlockSpec(memory_space=pl.ANY)
    out = pl.pallas_call(
        kernel,
        in_specs=[any_spec, any_spec, any_spec],
        out_specs=any_spec,
        out_shape=jax.ShapeDtypeStruct((NH, S, D), q.dtype),
        scratch_shapes=[
            pltpu.VMEM((NH, S, D), q.dtype),
            pltpu.VMEM((NH, S, D), k.dtype),
            pltpu.VMEM((NH, S, D), v.dtype),
            pltpu.VMEM((NH, S, D), q.dtype),
            pltpu.VMEM((KT, KT), jnp.float32),
            pltpu.VMEM((KT, KT), jnp.float32),
            pltpu.SemaphoreType.DMA((nch + 1,)),
            pltpu.SemaphoreType.DMA(()),
        ],
        compiler_params=pltpu.CompilerParams(
            vmem_limit_bytes=100 * 1024 * 1024),
    )(q3, k3, v3)
    return out.reshape(B, H, S, D)
```

```python
import functools
import math

import jax
import jax.numpy as jnp
from jax import lax
import jax.experimental.pallas as pl
import jax.experimental.pallas.tpu as pltpu

WINDOW = 32
KT = 128
TQ = KT - WINDOW
NEG = -1e30
WRITE_ROWS = 64
TAIL_ROWS = 1536


def _chunk_sizes(num_heads):
    n = num_heads // 4
    sizes = [n] * (num_heads // n)
    if num_heads % n:
        sizes.append(num_heads % n)
    return sizes


@jax.jit
def pallas_standalone__sliding_local_fixed_window__prompt_kernel(
    q: jax.Array,
    k: jax.Array,
    v: jax.Array,
):
    B, H, S, D = q.shape
    NH = B * H
    assert D == 128 and S >= KT and (S - KT) % TQ == 0 and S % WRITE_ROWS == 0
    assert S > TAIL_ROWS and NH >= 4
    q3, k3, v3 = (x.reshape(NH, S, D) for x in (q, k, v))

    chunks = _chunk_sizes(NH)
    nch = len(chunks)
    starts = [sum(chunks[:c]) for c in range(nch)]
    last0 = starts[-1]
    nblk = (S - KT) // TQ
    c1 = (D ** -0.5) * math.log2(math.e)

    def body(q_hbm, k_hbm, v_hbm, o_hbm, qb, kb, vb, ob, rsems, wsem):
        def read_copies(c):
            h0, n = starts[c], chunks[c]
            sem = rsems.at[c]
            hs = pl.ds(h0, n)
            cps = [pltpu.make_async_copy(q_hbm.at[hs], qb.at[hs], sem),
                   pltpu.make_async_copy(k_hbm.at[hs], kb.at[hs], sem)]
            if c < nch - 1:
                cps.append(pltpu.make_async_copy(v_hbm.at[hs], vb.at[hs], sem))
            else:
                if n > 1:
                    hs1 = pl.ds(h0, n - 1)
                    cps.append(
                        pltpu.make_async_copy(v_hbm.at[hs1], vb.at[hs1], sem))
                rs = pl.ds(0, S - TAIL_ROWS)
                cps.append(pltpu.make_async_copy(
                    v_hbm.at[NH - 1, rs], vb.at[NH - 1, rs], sem))
            return cps

        def tail_copy():
            rs = pl.ds(S - TAIL_ROWS, TAIL_ROWS)
            return pltpu.make_async_copy(
                v_hbm.at[NH - 1, rs], vb.at[NH - 1, rs], rsems.at[nch])

        def write_copies(h0, n):
            hs = pl.ds(h0, n)
            return [
                pltpu.make_async_copy(
                    ob.at[hs, pl.ds(j * WRITE_ROWS, WRITE_ROWS)],
                    o_hbm.at[hs, pl.ds(j * WRITE_ROWS, WRITE_ROWS)], wsem)
                for j in range(S // WRITE_ROWS)
            ]

        for c in range(nch):
            for cp in read_copies(c):
                cp.start()
        tail_copy().start()

        def arrive(c):
            for cp in read_copies(c):
                cp.wait()
            if c == nch - 1:
                for cp in write_copies(0, last0):
                    cp.start()
                tail_copy().wait()

        def block(h, q0, nq, k0):
            qq = qb[h, pl.ds(q0, nq), :]
            kk = kb[h, pl.ds(k0, KT), :]
            vv = vb[h, pl.ds(k0, KT), :]
            s = lax.dot_general(qq, kk, (((1,), (1,)), ((), ())),
                                preferred_element_type=jnp.float32)
            rel = (lax.broadcasted_iota(jnp.int32, (nq, KT), 0)
                   - lax.broadcasted_iota(jnp.int32, (nq, KT), 1)
                   + (q0 - k0))
            s = jnp.where((rel >= 0) & (rel < WINDOW), s, NEG)
            m = jnp.max(s, axis=-1, keepdims=True)
            p = jnp.exp2((s - m) * c1)
            l = jnp.sum(p, axis=-1, keepdims=True)
            o = jnp.dot(p.astype(vv.dtype), vv,
                        preferred_element_type=jnp.float32)
            ob[h, pl.ds(q0, nq), :] = (o / l).astype(ob.dtype)

        def head(h, carry):
            for c in range(nch):
                pl.when(h == starts[c])(functools.partial(arrive, c))
            block(h, 0, KT, 0)
            for j in range(nblk):
                q0 = KT + j * TQ
                block(h, q0, TQ, q0 - WINDOW)
            return carry

        lax.fori_loop(0, NH, head, 0)

        for cp in write_copies(last0, NH - last0):
            cp.start()
        for cp in write_copies(0, last0) + write_copies(last0, NH - last0):
            cp.wait()

    def kernel(*refs):
        pl.run_scoped(
            functools.partial(body, *refs),
            pltpu.SemaphoreType.DMA((nch + 1,)),
            pltpu.SemaphoreType.DMA(()),
        )

    any_spec = pl.BlockSpec(memory_space=pl.ANY)
    out = pl.pallas_call(
        kernel,
        in_specs=[any_spec, any_spec, any_spec],
        out_specs=any_spec,
        out_shape=jax.ShapeDtypeStruct((NH, S, D), q.dtype),
        scratch_shapes=[
            pltpu.VMEM((NH, S, D), q.dtype),
            pltpu.VMEM((NH, S, D), k.dtype),
            pltpu.VMEM((NH, S, D), v.dtype),
            pltpu.VMEM((NH, S, D), q.dtype),
        ],
        compiler_params=pltpu.CompilerParams(
            vmem_limit_bytes=100 * 1024 * 1024),
    )(q3, k3, v3)
    return out.reshape(B, H, S, D)
```

```python
import functools
import math

import jax
import jax.numpy as jnp
from jax import lax
import jax.experimental.pallas as pl
import jax.experimental.pallas.tpu as pltpu

WINDOW = 32
KT = 128
TQ = KT - WINDOW
NEG = -1e30
WRITE_ROWS = 64
TAIL_ROWS = 1536


def _chunk_sizes(num_heads):
    n = num_heads // 4
    sizes = [n] * (num_heads // n)
    if num_heads % n:
        sizes.append(num_heads % n)
    return sizes


@jax.jit
def pallas_standalone__sliding_local_fixed_window__prompt_kernel(
    q: jax.Array,
    k: jax.Array,
    v: jax.Array,
):
    B, H, S, D = q.shape
    NH = B * H
    assert D == 128 and S >= KT and (S - KT) % TQ == 0 and S % WRITE_ROWS == 0
    assert S > TAIL_ROWS and NH >= 4
    q3, k3, v3 = (x.reshape(NH, S, D) for x in (q, k, v))

    chunks = _chunk_sizes(NH)
    nch = len(chunks)
    starts = [sum(chunks[:c]) for c in range(nch)]
    last0 = starts[-1]
    nblk = (S - KT) // TQ
    c1 = (D ** -0.5) * math.log2(math.e)

    def body(q_hbm, k_hbm, v_hbm, o_hbm, qb, kb, vb, ob, bias0_ref, bias_ref,
             rsems, wsem):
        def read_copies(c):
            h0, n = starts[c], chunks[c]
            sem = rsems.at[c]
            hs = pl.ds(h0, n)
            cps = [pltpu.make_async_copy(q_hbm.at[hs], qb.at[hs], sem),
                   pltpu.make_async_copy(k_hbm.at[hs], kb.at[hs], sem)]
            if c < nch - 1:
                cps.append(pltpu.make_async_copy(v_hbm.at[hs], vb.at[hs], sem))
            else:
                if n > 1:
                    hs1 = pl.ds(h0, n - 1)
                    cps.append(
                        pltpu.make_async_copy(v_hbm.at[hs1], vb.at[hs1], sem))
                rs = pl.ds(0, S - TAIL_ROWS)
                cps.append(pltpu.make_async_copy(
                    v_hbm.at[NH - 1, rs], vb.at[NH - 1, rs], sem))
            return cps

        def tail_copy():
            rs = pl.ds(S - TAIL_ROWS, TAIL_ROWS)
            return pltpu.make_async_copy(
                v_hbm.at[NH - 1, rs], vb.at[NH - 1, rs], rsems.at[nch])

        def write_copies(h0, n):
            hs = pl.ds(h0, n)
            return [
                pltpu.make_async_copy(
                    ob.at[hs, pl.ds(j * WRITE_ROWS, WRITE_ROWS)],
                    o_hbm.at[hs, pl.ds(j * WRITE_ROWS, WRITE_ROWS)], wsem)
                for j in range(S // WRITE_ROWS)
            ]

        for c in range(nch):
            for cp in read_copies(c):
                cp.start()
        tail_copy().start()

        rel0 = (lax.broadcasted_iota(jnp.int32, (KT, KT), 0)
                - lax.broadcasted_iota(jnp.int32, (KT, KT), 1))
        bias0_ref[...] = jnp.where((rel0 >= 0) & (rel0 < WINDOW), 0.0, NEG)
        rel1 = rel0 + WINDOW
        bias_ref[...] = jnp.where((rel1 >= 0) & (rel1 < WINDOW), 0.0, NEG)

        def arrive(c):
            for cp in read_copies(c):
                cp.wait()
            if c == nch - 1:
                for cp in write_copies(0, last0):
                    cp.start()
                tail_copy().wait()

        def block(h, q0, nq, k0):
            qq = qb[h, pl.ds(q0, nq), :]
            kk = kb[h, pl.ds(k0, KT), :]
            vv = vb[h, pl.ds(k0, KT), :]
            s = lax.dot_general(qq, kk, (((1,), (1,)), ((), ())),
                                preferred_element_type=jnp.float32)
            s = s + (bias0_ref[...] if q0 == k0 else bias_ref[0:nq, :])
            m = jnp.max(s, axis=-1, keepdims=True)
            p = jnp.exp2((s - m) * c1)
            l = jnp.sum(p, axis=-1, keepdims=True)
            o = jnp.dot(p.astype(vv.dtype), vv,
                        preferred_element_type=jnp.float32)
            ob[h, pl.ds(q0, nq), :] = (o / l).astype(ob.dtype)

        def head(h, carry):
            for c in range(nch):
                pl.when(h == starts[c])(functools.partial(arrive, c))
            block(h, 0, KT, 0)
            for j in range(nblk):
                q0 = KT + j * TQ
                block(h, q0, TQ, q0 - WINDOW)
            return carry

        lax.fori_loop(0, NH, head, 0)

        for cp in write_copies(last0, NH - last0):
            cp.start()
        for cp in write_copies(0, last0) + write_copies(last0, NH - last0):
            cp.wait()

    def kernel(*refs):
        pl.run_scoped(
            functools.partial(body, *refs),
            pltpu.SemaphoreType.DMA((nch + 1,)),
            pltpu.SemaphoreType.DMA(()),
        )

    any_spec = pl.BlockSpec(memory_space=pl.ANY)
    out = pl.pallas_call(
        kernel,
        in_specs=[any_spec, any_spec, any_spec],
        out_specs=any_spec,
        out_shape=jax.ShapeDtypeStruct((NH, S, D), q.dtype),
        scratch_shapes=[
            pltpu.VMEM((NH, S, D), q.dtype),
            pltpu.VMEM((NH, S, D), k.dtype),
            pltpu.VMEM((NH, S, D), v.dtype),
            pltpu.VMEM((NH, S, D), q.dtype),
            pltpu.VMEM((KT, KT), jnp.float32),
            pltpu.VMEM((KT, KT), jnp.float32),
        ],
        compiler_params=pltpu.CompilerParams(
            vmem_limit_bytes=100 * 1024 * 1024),
    )(q3, k3, v3)
    return out.reshape(B, H, S, D)
```

```python
import functools
import math

import jax
import jax.numpy as jnp
import numpy as np
from jax import lax
import jax.experimental.pallas as pl
import jax.experimental.pallas.tpu as pltpu

WINDOW = 32
KT = 128
TQ = KT - WINDOW
NEG = -0.7 * float(np.finfo(np.float32).max)
LOG2E = math.log2(math.e)
WRITE_ROWS = 64
TAIL_ROWS = 1536


def _chunk_sizes(num_heads):
    n = num_heads // 4
    sizes = [n] * (num_heads // n)
    if num_heads % n:
        sizes.append(num_heads % n)
    return sizes


@jax.jit
def pallas_standalone__sliding_local_fixed_window__prompt_kernel(
    q: jax.Array,
    k: jax.Array,
    v: jax.Array,
):
    B, H, S, D = q.shape
    NH = B * H
    assert D == 128 and S >= KT and (S - KT) % TQ == 0 and S % WRITE_ROWS == 0
    assert S > TAIL_ROWS and NH >= 4
    q3, k3, v3 = (x.reshape(NH, S, D) for x in (q, k, v))

    chunks = _chunk_sizes(NH)
    nch = len(chunks)
    starts = [sum(chunks[:c]) for c in range(nch)]
    last0 = starts[-1]
    nblk = (S - KT) // TQ
    scale = float(np.asarray(D ** -0.5, dtype=q.dtype))

    def body(q_hbm, k_hbm, v_hbm, o_hbm, qb, kb, vb, ob, bias0_ref, bias_ref,
             rsems, wsem):
        def read_copies(c):
            h0, n = starts[c], chunks[c]
            sem = rsems.at[c]
            hs = pl.ds(h0, n)
            cps = [pltpu.make_async_copy(q_hbm.at[hs], qb.at[hs], sem),
                   pltpu.make_async_copy(k_hbm.at[hs], kb.at[hs], sem)]
            if c < nch - 1:
                cps.append(pltpu.make_async_copy(v_hbm.at[hs], vb.at[hs], sem))
            else:
                if n > 1:
                    hs1 = pl.ds(h0, n - 1)
                    cps.append(
                        pltpu.make_async_copy(v_hbm.at[hs1], vb.at[hs1], sem))
                rs = pl.ds(0, S - TAIL_ROWS)
                cps.append(pltpu.make_async_copy(
                    v_hbm.at[NH - 1, rs], vb.at[NH - 1, rs], sem))
            return cps

        def tail_copy():
            rs = pl.ds(S - TAIL_ROWS, TAIL_ROWS)
            return pltpu.make_async_copy(
                v_hbm.at[NH - 1, rs], vb.at[NH - 1, rs], rsems.at[nch])

        def write_copies(h0, n):
            hs = pl.ds(h0, n)
            return [
                pltpu.make_async_copy(
                    ob.at[hs, pl.ds(j * WRITE_ROWS, WRITE_ROWS)],
                    o_hbm.at[hs, pl.ds(j * WRITE_ROWS, WRITE_ROWS)], wsem)
                for j in range(S // WRITE_ROWS)
            ]

        for c in range(nch):
            for cp in read_copies(c):
                cp.start()
        tail_copy().start()

        def arrive(c):
            for cp in read_copies(c):
                cp.wait()
            if c == nch - 1:
                for cp in write_copies(0, last0):
                    cp.start()
                tail_copy().wait()

        rel0 = (lax.broadcasted_iota(jnp.int32, (KT, KT), 0)
                - lax.broadcasted_iota(jnp.int32, (KT, KT), 1))
        bias0_ref[...] = jnp.where((rel0 >= 0) & (rel0 < WINDOW), 0.0, NEG)
        rel1 = rel0 + WINDOW
        bias_ref[...] = jnp.where((rel1 >= 0) & (rel1 < WINDOW), 0.0, NEG)

        def block(h, q0, nq, k0, bias):
            qq = qb[h, pl.ds(q0, nq), :]
            kk = kb[h, pl.ds(k0, KT), :]
            vv = vb[h, pl.ds(k0, KT), :]
            s = lax.dot_general(qq, kk, (((1,), (1,)), ((), ())),
                                preferred_element_type=jnp.float32)
            s = s.astype(qq.dtype).astype(jnp.float32) * scale
            s = s.astype(qq.dtype).astype(jnp.float32)
            s = s + bias
            m = jnp.max(s, axis=-1, keepdims=True)
            p = jnp.exp2((s - m) * LOG2E)
            l = jnp.sum(p, axis=-1, keepdims=True)
            o = jnp.dot(p.astype(vv.dtype), vv,
                        preferred_element_type=jnp.float32)
            r = pl.reciprocal(l, approx=True)
            r = r * (2.0 - l * r)
            ob[h, pl.ds(q0, nq), :] = (o * r).astype(ob.dtype)

        def head(h, carry):
            for c in range(nch):
                pl.when(h == starts[c])(functools.partial(arrive, c))
            block(h, 0, KT, 0, bias0_ref[...])
            for j in range(nblk):
                q0 = KT + j * TQ
                block(h, q0, TQ, q0 - WINDOW, bias_ref[0:TQ, :])
            return carry

        lax.fori_loop(0, NH, head, 0)

        for cp in write_copies(last0, NH - last0):
            cp.start()
        for cp in write_copies(0, last0) + write_copies(last0, NH - last0):
            cp.wait()

    def kernel(*refs):
        pl.run_scoped(
            functools.partial(body, *refs),
            pltpu.SemaphoreType.DMA((nch + 1,)),
            pltpu.SemaphoreType.DMA(()),
        )

    any_spec = pl.BlockSpec(memory_space=pl.ANY)
    out = pl.pallas_call(
        kernel,
        in_specs=[any_spec, any_spec, any_spec],
        out_specs=any_spec,
        out_shape=jax.ShapeDtypeStruct((NH, S, D), q.dtype),
        scratch_shapes=[
            pltpu.VMEM((NH, S, D), q.dtype),
            pltpu.VMEM((NH, S, D), k.dtype),
            pltpu.VMEM((NH, S, D), v.dtype),
            pltpu.VMEM((NH, S, D), q.dtype),
            pltpu.VMEM((KT, KT), jnp.float32),
            pltpu.VMEM((KT, KT), jnp.float32),
        ],
        compiler_params=pltpu.CompilerParams(
            vmem_limit_bytes=100 * 1024 * 1024),
    )(q3, k3, v3)
    return out.reshape(B, H, S, D)
```
